```python
import os as _os
_os.environ.setdefault("JAX_PLATFORMS", "cpu")
import jax
import jax.numpy as jnp

def _softmax(x, axis=-1):
    return jax.nn.softmax(x, axis=axis)
def _gelu(x):
    return jax.nn.gelu(x, approximate=True)
def _silu(x):
    return jax.nn.silu(x)
def _sigmoid(x):
    return jax.nn.sigmoid(x)
def _layernorm(x, axis=-1, eps=1e-5):
    m = jnp.mean(x, axis=axis, keepdims=True)
    v = jnp.var(x, axis=axis, keepdims=True)
    return (x - m) / jnp.sqrt(v + eps)
def _scatter_add(tgt, idx, src, axis=0):
    return tgt.at[idx].add(src)
def _segment_sum(src, seg, n):
    return jax.ops.segment_sum(src, seg, n)
class _Rng:
    def __init__(self, key):
        self._k = key
    def _next(self):
        self._k, sub = jax.random.split(self._k)
        return sub
    def normal(self, shape):
        return jax.random.normal(self._next(), shape, dtype=jnp.bfloat16)
    def randint(self, lo, hi, shape):
        return jax.random.randint(self._next(), shape, lo, hi, dtype=jnp.int32)
    def uniform(self, shape, lo=0.0, hi=1.0):
        return jax.random.uniform(self._next(), shape, jnp.bfloat16, lo, hi)
    def permutation(self, n):
        return jax.random.permutation(self._next(), n)


kernel_name = 'interleave_layers__gqa_block_cached__dense_activation_silu__decode'

def setup_inputs():
    _rng = _Rng(jax.random.key(int.from_bytes(__import__("os").urandom(4), "little")))
    _w = (lambda a: (lambda t: t.astype(jnp.bfloat16) if jnp.issubdtype(t.dtype, jnp.floating) else t)(jnp.asarray(a)))
    def _A_setup():
        B, Sq, D = 2, 1, 512
        Hq, Hkv, Sk, Dh = 32, 8, 8192, 128
        assert Hq % Hkv == 0, (Hq, Hkv)
        return {
            "x": _w((lambda *s: _rng.normal(s) * 0.1)(B, Sq, D)),
            "k_cache": _w((lambda *s: _rng.normal(s) * 0.8)(B, Hkv, Sk, Dh)),
            "v_cache": _w((lambda *s: _rng.normal(s) * 1.6)(B, Hkv, Sk, Dh)),
            "wq": _w((lambda *s: _rng.normal(s) * 0.8)(D, Hq * Dh) * (D ** -0.5)),
            "wo": _w((lambda *s: _rng.normal(s) * 1.6)(Hq * Dh, D) * ((Hq * Dh) ** -0.5)),
        }
    _A_in = _A_setup()

    def _B_setup():
        B, S, D, F = 2, 1, 512, 1792
        return {
            "x": _w((lambda *s: _rng.normal(s) * 0.1)(B, S, D)),
            "w1": _w((lambda *s: _rng.normal(s) * 0.4)(D, F) * (D ** -0.5)),
            "w2": _w((lambda *s: _rng.normal(s) * 0.4)(F, D) * (F ** -0.5)),
        }
    _B_in = _B_setup()

    return {
        "A_x": _A_in["x"],
        "A_k_cache": _A_in["k_cache"],
        "A_v_cache": _A_in["v_cache"],
        "A_wq": _A_in["wq"],
        "A_wo": _A_in["wo"],
        "B_x": _B_in["x"],
        "B_w1": _B_in["w1"],
        "B_w2": _B_in["w2"],
    }

def reference(A_x, A_k_cache, A_v_cache, A_wq, A_wo, B_x, B_w1, B_w2):
    def _A_ref(x, k_cache, v_cache, wq, wo):
        B, Sq, D = x.shape
        Hq, Dh = 32, 128
        Hkv = k_cache.shape[1]
        rep = Hq // Hkv
        q = (lambda x, *d: x.transpose(*d))((x @ wq).reshape(B, Sq, Hq, Dh), 0, 2, 1, 3)
        k = jnp.repeat(k_cache, rep, axis=1)
        v = jnp.repeat(v_cache, rep, axis=1)
        scores = jnp.einsum("bhqd,bhkd->bhqk", q, k) * (Dh ** -0.5)
        p = _softmax(scores, axis=-1)
        o = jnp.einsum("bhqk,bhkd->bhqd", p, v)
        return (lambda x, *d: x.transpose(*d))(o, 0, 2, 1, 3).reshape(B, Sq, Hq * Dh) @ wo

    def _B_ref(x, w1, w2):
        h = jnp.einsum("bsd,df->bsf", x, w1)
        h = _silu(h)
        out = jnp.einsum("bsf,fd->bsd", h, w2)
        return out

    x = A_x
    x = x + _A_ref(_layernorm(x, axis=-1), A_k_cache, A_v_cache, A_wq, A_wo)
    x = x + _B_ref(_layernorm(x, axis=-1), B_w1, B_w2)
    x = x + _A_ref(_layernorm(x, axis=-1), A_k_cache, A_v_cache, A_wq, A_wo)
    x = x + _B_ref(_layernorm(x, axis=-1), B_w1, B_w2)
    return x
```

```python
import functools
import math
import jax
import jax.numpy as jnp
from jax import lax
import jax.experimental.pallas as pl
import jax.experimental.pallas.tpu as pltpu

B, D, HKV, REP, S, DH, F = 2, 512, 8, 4, 8192, 128, 1792
EPS = 1e-5
QSCALE = (DH ** -0.5) * math.log2(math.e)
NT = (((1,), (1,)), ((), ()))


def _ln(x):
    m = jnp.mean(x, axis=-1, keepdims=True)
    xc = x - m
    v = jnp.mean(xc * xc, axis=-1, keepdims=True)
    return (xc * lax.rsqrt(v + EPS)).astype(jnp.bfloat16)


def make(ahead=1, unroll_tail=False):
    NH = B * HKV
    def kernel(x_hbm, k_hbm, v_hbm, wq_hbm, wo_hbm, w1_hbm, w2_hbm, o_ref,
               xbuf, kbuf, vbuf, wq, wo, w1, w2, qbuf, sem_w, sem_k, sem_v):
        cx = pltpu.make_async_copy(x_hbm, xbuf, sem_w.at[0])
        cwq = pltpu.make_async_copy(wq_hbm, wq, sem_w.at[1])
        cwo = pltpu.make_async_copy(wo_hbm, wo, sem_w.at[2])
        cw1 = pltpu.make_async_copy(w1_hbm, w1, sem_w.at[3])
        cw2 = pltpu.make_async_copy(w2_hbm, w2, sem_w.at[4])
        ck = lambda j: pltpu.make_async_copy(k_hbm.at[j], kbuf.at[j], sem_k.at[j])
        cv = lambda j: pltpu.make_async_copy(v_hbm.at[j], vbuf.at[j], sem_v.at[j])
        cwq.start(); cx.start(); cwo.start(); cw1.start(); cw2.start()
        for j in range(ahead):
            ck(j).start(); cv(j).start()

        row = lax.broadcasted_iota(jnp.int32, (8, DH), 0)
        k32 = kbuf.bitcast(jnp.uint32)
        v32 = vbuf.bitcast(jnp.uint32)

        def qproj(x, b):
            h = _ln(x)
            for g in range(HKV):
                qa = jnp.dot(h, wq[:, g * 512:(g + 1) * 512], preferred_element_type=jnp.float32)
                qg = qa[:, 0:DH]
                for j in range(1, REP):
                    qg = jnp.where(row == j, qa[:, j * DH:(j + 1) * DH], qg)
                qbuf[b * HKV + g] = qg

        def head(b, g, acc, stream):
            j = b * HKV + g
            q = qbuf[j].astype(jnp.bfloat16)
            if stream:
                ck(j).wait()
                pl.when(j + ahead < NH)(lambda: ck(jnp.minimum(j + ahead, NH - 1)).start())
            kk = pltpu.bitcast(k32[j], jnp.bfloat16)
            s = lax.dot_general(q, kk, NT, preferred_element_type=jnp.float32) * QSCALE
            m = jnp.max(s, axis=-1, keepdims=True)
            p = jnp.exp2(s - m)
            l = jnp.sum(p, axis=-1, keepdims=True)
            if stream:
                cv(j).wait()
                pl.when(j + ahead < NH)(lambda: cv(jnp.minimum(j + ahead, NH - 1)).start())
            vv = pltpu.bitcast(v32[j], jnp.bfloat16)
            o = jnp.dot(p.astype(jnp.bfloat16), vv, preferred_element_type=jnp.float32) / l
            lhs = jnp.concatenate([jnp.where(row == r, o, 0.0) for r in range(REP)], axis=1)
            w = wo[pl.ds(pl.multiple_of(g * 512, 512), 512), :]
            return acc + jnp.dot(lhs.astype(jnp.bfloat16), w, preferred_element_type=jnp.float32)

        def ffn(x):
            h = jnp.dot(_ln(x), w1[...], preferred_element_type=jnp.float32)
            h = h * jax.nn.sigmoid(h)
            return jnp.dot(h.astype(jnp.bfloat16), w2[...], preferred_element_type=jnp.float32)

        z = jnp.zeros((8, D), jnp.float32)
        rs = lambda a: jnp.sum(a, axis=0, keepdims=True)
        cx.wait(); cwq.wait()
        xf = xbuf[...].astype(jnp.float32)
        x0 = jnp.broadcast_to(xf[0:1], (8, D))
        x1 = jnp.broadcast_to(xf[1:2], (8, D))
        qproj(x0, 0)
        qproj(x1, 1)
        cwo.wait()
        x0 = x0 + rs(lax.fori_loop(0, HKV, lambda g, a: head(0, g, a, True), z))
        cw1.wait(); cw2.wait()
        x0 = x0 + ffn(x0)
        qproj(x0, 0)
        def mid(g, c):
            return head(0, g, c[0], False), head(1, g, c[1], True)
        a0, a1 = lax.fori_loop(0, HKV - 1, mid, (z, z))
        a0 = head(0, HKV - 1, a0, False)
        x0 = x0 + rs(a0)
        x0 = x0 + ffn(x0)
        a1 = head(1, HKV - 1, a1, True)
        x1 = x1 + rs(a1)
        x1 = x1 + ffn(x1)
        qproj(x1, 1)
        if unroll_tail:
            a1 = z
            for g in range(HKV):
                a1 = head(1, g, a1, False)
        else:
            a1 = lax.fori_loop(0, HKV, lambda g, a: head(1, g, a, False), z)
        x1 = x1 + rs(a1)
        x1 = x1 + ffn(x1)
        r2 = lax.broadcasted_iota(jnp.int32, (B, D), 0)
        o_ref[...] = jnp.where(r2 == 0, x0[0:B], x1[0:B]).astype(o_ref.dtype)

    @jax.jit
    def f(A_x, A_k_cache, A_v_cache, A_wq, A_wo, B_x, B_w1, B_w2):
        hbm = pl.BlockSpec(memory_space=pltpu.HBM)
        bf = jnp.bfloat16
        out = pl.pallas_call(
            kernel,
            out_shape=jax.ShapeDtypeStruct((B, D), bf),
            in_specs=[hbm] * 7,
            out_specs=pl.BlockSpec(memory_space=pltpu.VMEM),
            scratch_shapes=[
                pltpu.VMEM((B, D), bf),
                pltpu.VMEM((NH, S, DH), bf), pltpu.VMEM((NH, S, DH), bf),
                pltpu.VMEM((D, HKV * REP * DH), bf), pltpu.VMEM((HKV * REP * DH, D), bf),
                pltpu.VMEM((D, F), bf), pltpu.VMEM((F, D), bf),
                pltpu.VMEM((NH, 8, DH), jnp.float32),
                pltpu.SemaphoreType.DMA((5,)), pltpu.SemaphoreType.DMA((NH,)), pltpu.SemaphoreType.DMA((NH,)),
            ],
            compiler_params=pltpu.CompilerParams(vmem_limit_bytes=100 * 1024 * 1024),
        )(A_x.reshape(B, D), A_k_cache.reshape(NH, S, DH), A_v_cache.reshape(NH, S, DH), A_wq, A_wo, B_w1, B_w2)
        return out.reshape(B, 1, D)
    return f


pallas_interleave_layers__gqa_block_cached__dense_activation_silu__decode_kernel = make(1, True)
```

```python
import functools
import math

import jax
import jax.numpy as jnp
from jax import lax
import jax.experimental.pallas as pl
import jax.experimental.pallas.tpu as pltpu

B, D, HKV, REP, S, DH, F = 2, 512, 8, 4, 8192, 128, 1792
NH = B * HKV
GW = REP * DH
EPS = 1e-5
QSCALE = (DH ** -0.5) * math.log2(math.e)
NT = (((1,), (1,)), ((), ()))
f32, bf16, u32 = jnp.float32, jnp.bfloat16, jnp.uint32

CUTS = (0, 3072, 6144, 7680, 8192)
CH = 512
NWO = 6
DELAY = 12


def _dot(a, b):
    return jnp.dot(a, b, preferred_element_type=f32)


def _ln(x):
    xc = x - jnp.mean(x, axis=-1, keepdims=True)
    var = jnp.mean(xc * xc, axis=-1, keepdims=True)
    return xc.astype(bf16), lax.rsqrt(var + EPS)


def _exp_sum(s):
    p = jnp.exp2(s - jnp.max(s, axis=-1, keepdims=True))
    return p, jnp.sum(p, axis=-1, keepdims=True)


def _kernel(x_hbm, k_hbm, v_hbm, wq_hbm, wo_hbm, w1_hbm, w2_hbm, o_ref,
            xbuf, kbuf, vbuf, ktbuf, wq, wo, w1, w2, qbuf, pbuf, lbuf,
            sem_w, sem_k, sem_v, sem_l):
    cx = pltpu.make_async_copy(x_hbm, xbuf, sem_w.at[0])
    cwq = pltpu.make_async_copy(wq_hbm, wq, sem_w.at[1])
    cwo = pltpu.make_async_copy(wo_hbm, wo, sem_w.at[2])
    cw1 = pltpu.make_async_copy(w1_hbm, w1, sem_w.at[3])
    cw2 = pltpu.make_async_copy(w2_hbm, w2, sem_w.at[4])
    ck = lambda j: pltpu.make_async_copy(k_hbm.at[j], kbuf.at[j], sem_k.at[j])
    cv = lambda j: pltpu.make_async_copy(v_hbm.at[j], vbuf.at[j], sem_v.at[j])

    def cl(c):
        piece = pl.ds(CUTS[c], CUTS[c + 1] - CUTS[c])
        return pltpu.make_async_copy(
            v_hbm.at[NH - 1, piece], vbuf.at[NH - 1, piece], sem_l.at[c])

    for c in (cwq, cx, ck(0), cv(0), cwo, ck(1), cv(1)):
        c.start()

    row = lax.broadcasted_iota(jnp.int32, (8, DH), 0)
    zero = jnp.zeros((8, D), f32)
    rowsum = lambda a: jnp.sum(a, axis=0, keepdims=True)

    def heads_to_rows(parts):
        q = parts[0]
        for j in range(1, REP):
            q = jnp.where(row == j, parts[j], q)
        return q

    def split_heads(qa):
        return heads_to_rows([qa[:, j * DH:(j + 1) * DH] for j in range(REP)])

    def qproj(x, b):
        h, r = _ln(x)
        qall = _dot(h, wq[...])
        for g in range(HKV):
            qbuf[b * HKV + g] = split_heads(qall[:, g * GW:(g + 1) * GW]) * (r * QSCALE)

    def oproj(o, g):
        lhs = jnp.concatenate([jnp.where(row == r, o, 0.0) for r in range(REP)], axis=1)
        start = g * GW if isinstance(g, int) else pl.multiple_of(g * GW, GW)
        return _dot(lhs.astype(bf16), wo[pl.ds(start, GW), :])

    def ffn(x):
        h, r = _ln(x)
        h = _dot(h, w1[...]) * r
        h = h * jax.nn.sigmoid(h)
        return _dot(h.astype(bf16), w2[...])

    def head0(g, acc, stream):
        q = qbuf[g].astype(bf16)
        if stream:
            ck(g).wait()
            ck(g + 2).start()
        p, l = _exp_sum(lax.dot_general(q, kbuf[g], NT, preferred_element_type=f32))
        if stream:
            cv(g).wait()
            pl.when(g + 2 < HKV)(lambda: cv(jnp.minimum(g + 2, HKV - 1)).start())
        return acc + oproj(_dot(p.astype(bf16), vbuf[g]) / l, g)

    ldk = lambda g, cols: pltpu.bitcast(ktbuf[g, :, cols], bf16)
    ldv = lambda j, r0, n: pltpu.bitcast(
        vbuf.bitcast(u32)[j, r0 // 2:(r0 + n) // 2, :], bf16)

    def kstage(g):
        j = HKV + g
        ck(j).wait()
        pl.when(g + 4 < HKV)(lambda: ck(jnp.minimum(j + 4, NH - 1)).start())
        pl.when(g + 4 >= HKV)(lambda: cv(jnp.maximum(j - 4, HKV)).start())
        ktbuf[g] = pltpu.bitcast(kbuf[j].T, u32)
        p, l = _exp_sum(_dot(qbuf[j].astype(bf16), ldk(g, slice(None))))
        pbuf[g] = (p * (1.0 / l)).astype(bf16)
        lbuf[g] = jnp.broadcast_to(l, (8, DH))

    def vstage(g, acc):
        cv(HKV + g).wait()
        return acc + oproj(_dot(pbuf[g], vbuf[HKV + g]), g)

    cx.wait()
    cwq.wait()
    xf = xbuf[...].astype(f32)
    x0 = jnp.broadcast_to(xf[0:1], (8, D))
    x1 = jnp.broadcast_to(xf[1:2], (8, D))
    qproj(x0, 0)
    qproj(x1, 1)
    cwo.wait()
    cw1.start()
    cw2.start()
    x0 = x0 + rowsum(lax.fori_loop(0, HKV, lambda g, a: head0(g, a, True), zero))
    ck(HKV + 2).start()
    ck(HKV + 3).start()
    cw1.wait()
    cw2.wait()
    x0 = x0 + ffn(x0)
    qproj(x0, 0)

    def step_a(g, a):
        kstage(g)
        return head0(g, a, False)

    def step_b(g, c):
        kstage(g)
        return c

    def step_c(g, accs):
        a1 = vstage(g, accs[1])
        pl.when(g < 3)(lambda: cv(jnp.minimum(HKV + 4 + g, NH - 2)).start())
        return head0(4 + g, accs[0], False), a1

    a0 = lax.fori_loop(0, 4, step_a, zero)
    lax.fori_loop(4, HKV, step_b, 0)
    a0, a1 = lax.fori_loop(0, 4, step_c, (a0, zero))
    for c in range(len(CUTS) - 1):
        cl(c).start()
    x0 = x0 + rowsum(a0)
    x0 = x0 + ffn(x0)
    a1 = lax.fori_loop(4, HKV - 1, vstage, a1)
    o = None
    for c in range(len(CUTS) - 1):
        cl(c).wait()
        t = _dot(pbuf[HKV - 1, :, CUTS[c]:CUTS[c + 1]],
                 ldv(NH - 1, CUTS[c], CUTS[c + 1] - CUTS[c]))
        o = t if o is None else o + t
    x1 = x1 + rowsum(a1 + oproj(o, HKV - 1))
    x1 = x1 + ffn(x1)

    h, r = _ln(x1)
    r = r * QSCALE

    def vpu_matvec(w_ref, r0, c0, col, acc):
        for k in range(0, col.shape[0], 16):
            for j in range(REP):
                w = w_ref[r0 + k:r0 + k + 16, c0 + j * DH:c0 + (j + 1) * DH]
                t = w.astype(f32) * col[k:k + 16]
                t = t[0:8] + t[8:16]
                acc[j] = t if acc[j] is None else acc[j] + t
            yield (acc[0] + acc[1]) + (acc[2] + acc[3])

    qs = {0: split_heads(_dot(h, wq[:, 0:GW])) * r}
    hcol = jnp.broadcast_to(h[0:1].astype(f32), (DH, D)).T

    def q_work():
        for g in range(1, HKV):
            acc = [None] * REP
            yield from vpu_matvec(wq, 0, g * GW, hcol, acc)
            qs[g] = heads_to_rows([jnp.broadcast_to(rowsum(a), (8, DH)) for a in acc]) * r

    q_steps = q_work()
    oacc = [None] * REP
    o_tasks = []
    clock = [0]

    def o_work(cols, g):
        for j in range(REP):
            yield from vpu_matvec(wo, g * GW + j * DH, 0, cols[j], oacc)

    def o_step():
        while o_tasks and clock[0] >= o_tasks[0][0]:
            d = next(o_tasks[0][1], None)
            if d is not None:
                return d
            o_tasks.pop(0)
        return None

    never = lbuf[0] < 0.0
    pending = [None]

    def tick(v):
        clock[0] += 1
        done = []
        for _ in range(2):
            d = next(q_steps, None)
            d = o_step() if d is None else d
            if d is not None:
                done.append(d)
        pending.append(functools.reduce(jnp.add, done) if done else None)
        d = pending.pop(0)
        return v if d is None else jnp.where(never, d, v)

    def scores(g):
        while g not in qs:
            next(q_steps, None)
        return [_dot(tick(qs[g]).astype(bf16), ldk(g, slice(c, c + CH)))
                for c in range(0, S, CH)]

    def attend(g, s):
        tiles = lambda a: [a[:, j:j + DH] for j in range(0, CH, DH)]
        m = functools.reduce(jnp.maximum, [t for a in s for t in tiles(a)])
        m = jnp.broadcast_to(jnp.max(m, axis=-1, keepdims=True), (8, DH))
        o = l = None
        for c in range(S // CH):
            p = jnp.exp2(s[c] - jnp.concatenate([tick(m)] * (CH // DH), axis=1))
            lc = functools.reduce(jnp.add, tiles(p))
            l = lc if l is None else l + lc
            t = _dot(p.astype(bf16), ldv(HKV + g, c * CH, CH))
            o = t if o is None else o + t
        return o / jnp.sum(l, axis=-1, keepdims=True)

    a1 = zero
    s = scores(0)
    for g in range(HKV):
        s_next = scores(g + 1) if g + 1 < HKV else None
        o_new = attend(g, s)
        if g < NWO:
            cols = [jnp.broadcast_to(o_new[j:j + 1], (DH, DH)).T for j in range(REP)]
            o_tasks.append((clock[0] + DELAY, o_work(cols, g)))
        if g > NWO:
            a1 = a1 + oproj(o, g - 1)
        o, s = o_new, s_next
    a1 = a1 + oproj(o, HKV - 1)
    clock[0] += DELAY
    while o_step() is not None:
        pass
    x1 = x1 + rowsum(a1 + jnp.concatenate(oacc, axis=1))
    x1 = x1 + ffn(x1)

    which = lax.broadcasted_iota(jnp.int32, (B, D), 0)
    o_ref[...] = jnp.where(which == 0, x0[0:B], x1[0:B]).astype(o_ref.dtype)


@jax.jit
def pallas_interleave_layers__gqa_block_cached__dense_activation_silu__decode_kernel(
    A_x: jax.Array,
    A_k_cache: jax.Array,
    A_v_cache: jax.Array,
    A_wq: jax.Array,
    A_wo: jax.Array,
    B_x: jax.Array,
    B_w1: jax.Array,
    B_w2: jax.Array,
):
    del B_x
    out = pl.pallas_call(
        _kernel,
        out_shape=jax.ShapeDtypeStruct((B, D), A_x.dtype),
        in_specs=[pl.BlockSpec(memory_space=pltpu.HBM)] * 7,
        out_specs=pl.BlockSpec(memory_space=pltpu.VMEM),
        scratch_shapes=[
            pltpu.VMEM((B, D), bf16),
            pltpu.VMEM((NH, S, DH), bf16),
            pltpu.VMEM((NH, S, DH), bf16),
            pltpu.VMEM((HKV, DH // 2, S), u32),
            pltpu.VMEM((D, HKV * GW), bf16),
            pltpu.VMEM((HKV * GW, D), bf16),
            pltpu.VMEM((D, F), bf16),
            pltpu.VMEM((F, D), bf16),
            pltpu.VMEM((NH, 8, DH), f32),
            pltpu.VMEM((HKV, 8, S), bf16),
            pltpu.VMEM((HKV, 8, DH), f32),
            pltpu.SemaphoreType.DMA((5,)),
            pltpu.SemaphoreType.DMA((NH,)),
            pltpu.SemaphoreType.DMA((NH,)),
            pltpu.SemaphoreType.DMA((len(CUTS) - 1,)),
        ],
        compiler_params=pltpu.CompilerParams(vmem_limit_bytes=112 * 1024 * 1024),
    )(A_x.reshape(B, D), A_k_cache.reshape(NH, S, DH), A_v_cache.reshape(NH, S, DH),
      A_wq, A_wo, B_w1, B_w2)
    return out.reshape(B, 1, D)
```

```python
import functools
import math

import jax
import jax.numpy as jnp
from jax import lax
import jax.experimental.pallas as pl
import jax.experimental.pallas.tpu as pltpu

B, D, HKV, REP, S, DH, F = 2, 512, 8, 4, 8192, 128, 1792
NH = B * HKV
GW = REP * DH
EPS = 1e-5
QSCALE = (DH ** -0.5) * math.log2(math.e)
NT = (((1,), (1,)), ((), ()))
f32, bf16, u32 = jnp.float32, jnp.bfloat16, jnp.uint32

CUTS = (0, 3072, 6144, 7680, 8192)
CH = 512
NWO = 6
DELAY = 12


def _dot(a, b):
    return jnp.dot(a, b, preferred_element_type=f32)


def _ln(x):
    xc = x - jnp.mean(x, axis=-1, keepdims=True)
    var = jnp.mean(xc * xc, axis=-1, keepdims=True)
    return xc.astype(bf16), lax.rsqrt(var + EPS)


def _exp_sum(s):
    p = jnp.exp2(s - jnp.max(s, axis=-1, keepdims=True))
    return p, jnp.sum(p, axis=-1, keepdims=True)


def _kernel(x_hbm, k_hbm, v_hbm, wq_hbm, wo_hbm, w1_hbm, w2_hbm, o_ref,
            xbuf, kbuf, vbuf, ktbuf, wq, wo, w1, w2, qbuf, pbuf, lbuf,
            sem_w, sem_k, sem_v, sem_l):
    cx = pltpu.make_async_copy(x_hbm, xbuf, sem_w.at[0])
    cwq = pltpu.make_async_copy(wq_hbm, wq, sem_w.at[1])
    cwo = pltpu.make_async_copy(wo_hbm, wo, sem_w.at[2])
    cw1 = pltpu.make_async_copy(w1_hbm, w1, sem_w.at[3])
    cw2 = pltpu.make_async_copy(w2_hbm, w2, sem_w.at[4])
    ck = lambda j: pltpu.make_async_copy(k_hbm.at[j], kbuf.at[j], sem_k.at[j])
    cv = lambda j: pltpu.make_async_copy(v_hbm.at[j], vbuf.at[j], sem_v.at[j])

    def cl(c):
        piece = pl.ds(CUTS[c], CUTS[c + 1] - CUTS[c])
        return pltpu.make_async_copy(
            v_hbm.at[NH - 1, piece], vbuf.at[NH - 1, piece], sem_l.at[c])

    for c in (cwq, cx, ck(0), cv(0), cwo, ck(1), cv(1)):
        c.start()

    row = lax.broadcasted_iota(jnp.int32, (8, DH), 0)
    zero = jnp.zeros((8, D), f32)
    rowsum = lambda a: jnp.sum(a, axis=0, keepdims=True)

    def heads_to_rows(parts):
        q = parts[0]
        for j in range(1, REP):
            q = jnp.where(row == j, parts[j], q)
        return q

    def split_heads(qa):
        return heads_to_rows([qa[:, j * DH:(j + 1) * DH] for j in range(REP)])

    def qproj(x, b):
        h, r = _ln(x)
        qall = _dot(h, wq[...])
        for g in range(HKV):
            qbuf[b * HKV + g] = split_heads(qall[:, g * GW:(g + 1) * GW]) * (r * QSCALE)

    def oproj(o, g):
        lhs = jnp.concatenate([jnp.where(row == r, o, 0.0) for r in range(REP)], axis=1)
        start = g * GW if isinstance(g, int) else pl.multiple_of(g * GW, GW)
        return _dot(lhs.astype(bf16), wo[pl.ds(start, GW), :])

    def ffn(x):
        h, r = _ln(x)
        h = _dot(h, w1[...]) * r
        h = h * jax.nn.sigmoid(h)
        return _dot(h.astype(bf16), w2[...])

    def head0(g, acc, stream):
        q = qbuf[g].astype(bf16)
        if stream:
            ck(g).wait()
            ck(g + 2).start()
        p, l = _exp_sum(lax.dot_general(q, kbuf[g], NT, preferred_element_type=f32))
        if stream:
            cv(g).wait()
            pl.when(g + 2 < HKV)(lambda: cv(jnp.minimum(g + 2, HKV - 1)).start())
        return acc + oproj(_dot(p.astype(bf16), vbuf[g]) / l, g)

    ldk = lambda g, cols: pltpu.bitcast(ktbuf[g, :, cols], bf16)

    def kstage(g):
        j = HKV + g
        ck(j).wait()
        pl.when(g + 4 < HKV)(lambda: ck(jnp.minimum(j + 4, NH - 1)).start())
        pl.when(g + 4 >= HKV)(lambda: cv(jnp.maximum(j - 4, HKV)).start())
        ktbuf[g] = pltpu.bitcast(kbuf[j].T, u32)
        p, l = _exp_sum(_dot(qbuf[j].astype(bf16), ldk(g, slice(None))))
        pbuf[g] = (p * (1.0 / l)).astype(bf16)
        lbuf[g] = jnp.broadcast_to(l, (8, DH))

    def vstage(g, acc):
        cv(HKV + g).wait()
        return acc + oproj(_dot(pbuf[g], vbuf[HKV + g]), g)

    cx.wait()
    cwq.wait()
    xf = xbuf[...].astype(f32)
    x0 = jnp.broadcast_to(xf[0:1], (8, D))
    x1 = jnp.broadcast_to(xf[1:2], (8, D))
    qproj(x0, 0)
    qproj(x1, 1)
    cwo.wait()
    cw1.start()
    cw2.start()
    x0 = x0 + rowsum(lax.fori_loop(0, HKV, lambda g, a: head0(g, a, True), zero))
    ck(HKV + 2).start()
    ck(HKV + 3).start()
    cw1.wait()
    cw2.wait()
    x0 = x0 + ffn(x0)
    qproj(x0, 0)

    def step_a(g, a):
        kstage(g)
        return head0(g, a, False)

    def step_b(g, c):
        kstage(g)
        return c

    def step_c(g, accs):
        a1 = vstage(g, accs[1])
        pl.when(g < 3)(lambda: cv(jnp.minimum(HKV + 4 + g, NH - 2)).start())
        return head0(4 + g, accs[0], False), a1

    a0 = lax.fori_loop(0, 4, step_a, zero)
    lax.fori_loop(4, HKV, step_b, 0)
    a0, a1 = lax.fori_loop(0, 4, step_c, (a0, zero))
    for c in range(len(CUTS) - 1):
        cl(c).start()
    x0 = x0 + rowsum(a0)
    x0 = x0 + ffn(x0)
    a1 = lax.fori_loop(4, HKV - 1, vstage, a1)
    o = None
    for c in range(len(CUTS) - 1):
        cl(c).wait()
        t = _dot(pbuf[HKV - 1, :, CUTS[c]:CUTS[c + 1]],
                 vbuf[NH - 1, CUTS[c]:CUTS[c + 1], :])
        o = t if o is None else o + t
    x1 = x1 + rowsum(a1 + oproj(o, HKV - 1))
    x1 = x1 + ffn(x1)

    h, r = _ln(x1)
    r = r * QSCALE

    def vpu_matvec(w_ref, r0, c0, col, acc):
        for k in range(0, col.shape[0], 16):
            for j in range(REP):
                w = w_ref[r0 + k:r0 + k + 16, c0 + j * DH:c0 + (j + 1) * DH]
                t = w.astype(f32) * col[k:k + 16]
                t = t[0:8] + t[8:16]
                acc[j] = t if acc[j] is None else acc[j] + t
            yield (acc[0] + acc[1]) + (acc[2] + acc[3])

    qs = {0: split_heads(_dot(h, wq[:, 0:GW])) * r}
    hcol = jnp.broadcast_to(h[0:1].astype(f32), (DH, D)).T

    def q_work():
        for g in range(1, HKV):
            acc = [None] * REP
            yield from vpu_matvec(wq, 0, g * GW, hcol, acc)
            qs[g] = heads_to_rows([jnp.broadcast_to(rowsum(a), (8, DH)) for a in acc]) * r

    q_steps = q_work()
    oacc = [None] * REP
    o_tasks = []
    clock = [0]

    def o_work(cols, g):
        for j in range(REP):
            yield from vpu_matvec(wo, g * GW + j * DH, 0, cols[j], oacc)

    def o_step():
        while o_tasks and clock[0] >= o_tasks[0][0]:
            d = next(o_tasks[0][1], None)
            if d is not None:
                return d
            o_tasks.pop(0)
        return None

    never = lbuf[0] < 0.0
    pending = [None]

    def tick(v):
        clock[0] += 1
        done = []
        for _ in range(2):
            d = next(q_steps, None)
            d = o_step() if d is None else d
            if d is not None:
                done.append(d)
        pending.append(functools.reduce(jnp.add, done) if done else None)
        d = pending.pop(0)
        return v if d is None else jnp.where(never, d, v)

    def scores(g):
        while g not in qs:
            next(q_steps, None)
        return [_dot(tick(qs[g]).astype(bf16), ldk(g, slice(c, c + CH)))
                for c in range(0, S, CH)]

    def attend(g, s):
        tiles = lambda a: [a[:, j:j + DH] for j in range(0, CH, DH)]
        m = functools.reduce(jnp.maximum, [t for a in s for t in tiles(a)])
        m = jnp.broadcast_to(jnp.max(m, axis=-1, keepdims=True), (8, DH))
        o = l = None
        for c in range(S // CH):
            p = jnp.exp2(s[c] - jnp.concatenate([tick(m)] * (CH // DH), axis=1))
            lc = functools.reduce(jnp.add, tiles(p))
            l = lc if l is None else l + lc
            t = _dot(p.astype(bf16), vbuf[HKV + g, c * CH:(c + 1) * CH, :])
            o = t if o is None else o + t
        return o / jnp.sum(l, axis=-1, keepdims=True)

    a1 = zero
    s = scores(0)
    for g in range(HKV):
        s_next = scores(g + 1) if g + 1 < HKV else None
        o_new = attend(g, s)
        if g < NWO:
            cols = [jnp.broadcast_to(o_new[j:j + 1], (DH, DH)).T for j in range(REP)]
            o_tasks.append((clock[0] + DELAY, o_work(cols, g)))
        if g > NWO:
            a1 = a1 + oproj(o, g - 1)
        o, s = o_new, s_next
    a1 = a1 + oproj(o, HKV - 1)
    clock[0] += DELAY
    while o_step() is not None:
        pass
    x1 = x1 + rowsum(a1 + jnp.concatenate(oacc, axis=1))
    x1 = x1 + ffn(x1)

    which = lax.broadcasted_iota(jnp.int32, (B, D), 0)
    o_ref[...] = jnp.where(which == 0, x0[0:B], x1[0:B]).astype(o_ref.dtype)


@jax.jit
def pallas_interleave_layers__gqa_block_cached__dense_activation_silu__decode_kernel(
    A_x: jax.Array,
    A_k_cache: jax.Array,
    A_v_cache: jax.Array,
    A_wq: jax.Array,
    A_wo: jax.Array,
    B_x: jax.Array,
    B_w1: jax.Array,
    B_w2: jax.Array,
):
    del B_x
    out = pl.pallas_call(
        _kernel,
        out_shape=jax.ShapeDtypeStruct((B, D), A_x.dtype),
        in_specs=[pl.BlockSpec(memory_space=pltpu.HBM)] * 7,
        out_specs=pl.BlockSpec(memory_space=pltpu.VMEM),
        scratch_shapes=[
            pltpu.VMEM((B, D), bf16),
            pltpu.VMEM((NH, S, DH), bf16),
            pltpu.VMEM((NH, S, DH), bf16),
            pltpu.VMEM((HKV, DH // 2, S), u32),
            pltpu.VMEM((D, HKV * GW), bf16),
            pltpu.VMEM((HKV * GW, D), bf16),
            pltpu.VMEM((D, F), bf16),
            pltpu.VMEM((F, D), bf16),
            pltpu.VMEM((NH, 8, DH), f32),
            pltpu.VMEM((HKV, 8, S), bf16),
            pltpu.VMEM((HKV, 8, DH), f32),
            pltpu.SemaphoreType.DMA((5,)),
            pltpu.SemaphoreType.DMA((NH,)),
            pltpu.SemaphoreType.DMA((NH,)),
            pltpu.SemaphoreType.DMA((len(CUTS) - 1,)),
        ],
        compiler_params=pltpu.CompilerParams(vmem_limit_bytes=112 * 1024 * 1024),
    )(A_x.reshape(B, D), A_k_cache.reshape(NH, S, DH), A_v_cache.reshape(NH, S, DH),
      A_wq, A_wo, B_w1, B_w2)
    return out.reshape(B, 1, D)
```
